```python
import os as _os
_os.environ.setdefault("JAX_PLATFORMS", "cpu")
import jax
import jax.numpy as jnp

def _softmax(x, axis=-1):
    return jax.nn.softmax(x, axis=axis)
def _gelu(x):
    return jax.nn.gelu(x, approximate=True)
def _silu(x):
    return jax.nn.silu(x)
def _sigmoid(x):
    return jax.nn.sigmoid(x)
def _layernorm(x, axis=-1, eps=1e-5):
    m = jnp.mean(x, axis=axis, keepdims=True)
    v = jnp.var(x, axis=axis, keepdims=True)
    return (x - m) / jnp.sqrt(v + eps)
def _scatter_add(tgt, idx, src, axis=0):
    return tgt.at[idx].add(src)
def _segment_sum(src, seg, n):
    return jax.ops.segment_sum(src, seg, n)
class _Rng:
    def __init__(self, key):
        self._k = key
    def _next(self):
        self._k, sub = jax.random.split(self._k)
        return sub
    def normal(self, shape):
        return jax.random.normal(self._next(), shape, dtype=jnp.bfloat16)
    def randint(self, lo, hi, shape):
        return jax.random.randint(self._next(), shape, lo, hi, dtype=jnp.int32)
    def uniform(self, shape, lo=0.0, hi=1.0):
        return jax.random.uniform(self._next(), shape, jnp.bfloat16, lo, hi)
    def permutation(self, n):
        return jax.random.permutation(self._next(), n)


kernel_name = 'standalone__grn__sampling'

def setup_inputs():
    _rng = _Rng(jax.random.key(int.from_bytes(__import__("os").urandom(4), "little")))
    _w = (lambda a: (lambda t: t.astype(jnp.bfloat16) if jnp.issubdtype(t.dtype, jnp.floating) else t)(jnp.asarray(a)))
    B, S, D = 512, 32, 640
    return {
        "x": _w((lambda *s: _rng.normal(s) * 0.05)(B, S, D)),
        "g": _w((lambda *s: _rng.normal(s) * 0.1)(D) * 0.1),
        "b": _w((lambda *s: _rng.normal(s) * 0.1)(D) * 0.1),
    }

def reference(x, g, b):
    gx = jnp.sqrt((x * x).sum(axis=-2, keepdims=True))
    nx = gx / (gx.mean(axis=-1, keepdims=True) + 1e-6)
    return g * (x * nx) + b + x
```

```python
import jax
import jax.numpy as jnp
import jax.experimental.pallas as pl
import jax.experimental.pallas.tpu as pltpu

_K = 64
_RG = 4
_PRE = 8


def _grn_kernel(x_hbm, g_hbm, b_hbm, o_hbm, buf, gbuf, bbuf, rsem, wsem, psem):
    N, K, S, D = buf.shape
    NR = K // _RG

    def read(i):
        cols = pl.ds(i * _RG, _RG)
        return pltpu.make_async_copy(x_hbm.at[:, cols], buf.at[:, cols], rsem.at[i])

    def write(j):
        return pltpu.make_async_copy(buf.at[:, j], o_hbm.at[:, j], wsem)

    g_copy = pltpu.make_async_copy(g_hbm, gbuf, psem.at[0])
    b_copy = pltpu.make_async_copy(b_hbm, bbuf, psem.at[1])
    read(0).start()
    g_copy.start()
    b_copy.start()
    jax.lax.fori_loop(1, NR, lambda i, _: read(i).start(), None)
    g_copy.wait()
    b_copy.wait()
    gv = gbuf[...].astype(jnp.float32).reshape(1, D)
    bv = bbuf[...].astype(jnp.float32).reshape(1, D)

    def normalize(j):
        for n in range(N):
            xv = buf[n, j].astype(jnp.float32)
            gx = jnp.sqrt(jnp.sum(xv * xv, axis=0, keepdims=True))
            den = jnp.sum(gx, axis=-1, keepdims=True) * (1.0 / D) + 1e-6
            scale = gv * (gx / den) + 1.0
            buf[n, j] = (xv * scale + bv).astype(buf.dtype)

    def read_step(i, _):
        read(i).wait()
        jax.lax.fori_loop(0, _RG, lambda t, _: normalize(i * _RG + t), None)

    jax.lax.fori_loop(0, NR - 1, read_step, None)
    read(NR - 1).wait()
    jax.lax.fori_loop(0, _PRE, lambda j, _: write(j).start(), None)
    jax.lax.fori_loop(K - _RG, K, lambda j, _: normalize(j), None)
    jax.lax.fori_loop(_PRE, K, lambda j, _: write(j).start(), None)
    pltpu.make_async_copy(buf, buf, wsem).wait()


@jax.jit
def pallas_standalone__grn__sampling_kernel(
    x: jax.Array,
    g: jax.Array,
    b: jax.Array,
):
    B, S, D = x.shape
    shape = (B // _K, _K, S, D)
    out = pl.pallas_call(
        _grn_kernel,
        in_specs=[pl.BlockSpec(memory_space=pl.ANY)] * 3,
        out_specs=pl.BlockSpec(memory_space=pl.ANY),
        out_shape=jax.ShapeDtypeStruct(shape, x.dtype),
        scratch_shapes=[
            pltpu.VMEM(shape, x.dtype),
            pltpu.VMEM((D,), g.dtype),
            pltpu.VMEM((D,), b.dtype),
            pltpu.SemaphoreType.DMA((_K // _RG,)),
            pltpu.SemaphoreType.DMA(()),
            pltpu.SemaphoreType.DMA((2,)),
        ],
        compiler_params=pltpu.CompilerParams(vmem_limit_bytes=64 * 1024 * 1024),
    )(x.reshape(shape), g, b)
    return out.reshape(x.shape)
```

```python
import functools

import jax
import jax.numpy as jnp
import jax.experimental.pallas as pl
import jax.experimental.pallas.tpu as pltpu

_STREAMS = 8
_READ_COLS = 3
_LATE_COLS = 10
_WRITE_ROWS = 16
_WRITE_AHEAD = 16
_EPS = 1e-6


def _grn_kernel(x_hbm, g_hbm, b_hbm, o_hbm, buf, g_buf, b_buf, write_sem, *, seq):
    streams, rows, dim = buf.shape
    cols = rows // seq
    early_cols = cols - _LATE_COLS
    early_reads = early_cols // _READ_COLS
    num_writes = rows // _WRITE_ROWS
    writes_per_col = (early_cols * seq // _WRITE_ROWS - _WRITE_AHEAD) // _LATE_COLS

    def start_writes(first, count):
        def start(t, _):
            r = pl.ds(pl.multiple_of((first + t) * _WRITE_ROWS, _WRITE_ROWS), _WRITE_ROWS)
            pltpu.make_async_copy(buf.at[:, r], o_hbm.at[:, r], write_sem).start()

        jax.lax.fori_loop(0, count, start, None)

    def read_and_normalize(early_sems, late_sems, param_sems):
        def early_read(i):
            size = _READ_COLS * seq
            r = pl.ds(pl.multiple_of(i * size, size), size)
            return pltpu.make_async_copy(x_hbm.at[:, r], buf.at[:, r], early_sems.at[i])

        def late_read(slabs, k):
            r = pl.ds(early_cols * seq, _LATE_COLS * seq)
            return pltpu.make_async_copy(
                x_hbm.at[slabs, r], buf.at[slabs, r], late_sems.at[k]
            )

        late_head = late_read(pl.ds(0, streams - 1), 0)
        late_tail = late_read(pl.ds(streams - 1, 1), 1)
        g_read = pltpu.make_async_copy(g_hbm, g_buf, param_sems.at[0])
        b_read = pltpu.make_async_copy(b_hbm, b_buf, param_sems.at[1])

        early_read(0).start()
        g_read.start()
        b_read.start()
        jax.lax.fori_loop(1, early_reads, lambda i, _: early_read(i).start(), None)
        late_head.start()
        g_read.wait()
        b_read.wait()
        late_tail.start()
        g = g_buf[...].astype(jnp.float32).reshape(1, dim)
        b = b_buf[...].astype(jnp.float32).reshape(1, dim)

        def column(j, _):
            @pl.when(jnp.logical_and(j < early_cols, j % _READ_COLS == 0))
            def _():
                early_read(j // _READ_COLS).wait()

            @pl.when(j == early_cols)
            def _():
                late_head.wait()
                start_writes(0, _WRITE_AHEAD)
                late_tail.wait()

            r = pl.ds(pl.multiple_of(j * seq, seq), seq)
            for n in range(streams):
                x = buf[n, r].astype(jnp.float32)
                gx = jnp.sqrt(jnp.sum(x * x, axis=0, keepdims=True))
                nx = gx / (jnp.mean(gx, axis=-1, keepdims=True) + _EPS)
                buf[n, r] = (g * (x * nx) + b + x).astype(buf.dtype)

            @pl.when(j >= early_cols)
            def _():
                first = _WRITE_AHEAD + (j - early_cols) * writes_per_col
                start_writes(first, writes_per_col)

        jax.lax.fori_loop(0, cols, column, None)

    pl.run_scoped(
        read_and_normalize,
        pltpu.SemaphoreType.DMA((early_reads,)),
        pltpu.SemaphoreType.DMA((2,)),
        pltpu.SemaphoreType.DMA((2,)),
    )
    started = _WRITE_AHEAD + _LATE_COLS * writes_per_col
    start_writes(started, num_writes - started)
    pltpu.make_async_copy(buf, o_hbm, write_sem).wait()


@jax.jit
def pallas_standalone__grn__sampling_kernel(
    x: jax.Array,
    g: jax.Array,
    b: jax.Array,
):
    batch, seq, dim = x.shape
    assert batch % _STREAMS == 0 and seq % _WRITE_ROWS == 0
    early_cols = batch // _STREAMS - _LATE_COLS
    assert early_cols % _READ_COLS == 0
    assert early_cols * seq // _WRITE_ROWS >= _WRITE_AHEAD
    slabs = (_STREAMS, batch // _STREAMS * seq, dim)

    out = pl.pallas_call(
        functools.partial(_grn_kernel, seq=seq),
        in_specs=[pl.BlockSpec(memory_space=pl.ANY)] * 3,
        out_specs=pl.BlockSpec(memory_space=pl.ANY),
        out_shape=jax.ShapeDtypeStruct(slabs, x.dtype),
        scratch_shapes=[
            pltpu.VMEM(slabs, x.dtype),
            pltpu.VMEM((dim,), g.dtype),
            pltpu.VMEM((dim,), b.dtype),
            pltpu.SemaphoreType.DMA(()),
        ],
        compiler_params=pltpu.CompilerParams(vmem_limit_bytes=48 * 1024 * 1024),
    )(x.reshape(slabs), g, b)
    return out.reshape(x.shape)
```
